```python
import os as _os
_os.environ.setdefault('JAX_PLATFORMS', 'cpu')
import jax
import jax.numpy as jnp

def _softmax(x, axis=-1):
    return jax.nn.softmax(x, axis=axis)

def _gelu(x):
    return jax.nn.gelu(x, approximate=True)

def _silu(x):
    return jax.nn.silu(x)

def _sigmoid(x):
    return jax.nn.sigmoid(x)

def _layernorm(x, axis=-1, eps=1e-05):
    m = jnp.mean(x, axis=axis, keepdims=True)
    v = jnp.var(x, axis=axis, keepdims=True)
    return (x - m) / jnp.sqrt(v + eps)

def _scatter_add(tgt, idx, src, axis=0):
    return tgt.at[idx].add(src)

def _segment_sum(src, seg, n):
    return jax.ops.segment_sum(src, seg, n)

class _Rng:

    def __init__(self, key):
        self._k = key

    def _next(self):
        self._k, sub = jax.random.split(self._k)
        return sub

    def normal(self, shape):
        return jax.random.normal(self._next(), shape, dtype=jnp.bfloat16)

    def randint(self, lo, hi, shape):
        return jax.random.randint(self._next(), shape, lo, hi, dtype=jnp.int32)

    def uniform(self, shape, lo=0.0, hi=1.0):
        return jax.random.uniform(self._next(), shape, jnp.bfloat16, lo, hi)

    def permutation(self, n):
        return jax.random.permutation(self._next(), n)
kernel_name = 'gated_mix__mha_block__memory_aug_recurrent_mem_tr__prompt'

def setup_inputs():
    _rng = _Rng(jax.random.key(int.from_bytes(__import__("os").urandom(4), "little")))
    _w = lambda a: (lambda t: t.astype(jnp.bfloat16) if jnp.issubdtype(t.dtype, jnp.floating) else t)(jnp.asarray(a))

    def _A_setup():
        B, S, D, H = (1, 2048, 512, 32)
        return {'x': _w((lambda *s: _rng.normal(s) * 0.05)(B, S, D)), 'wqkv': _w((lambda *s: _rng.normal(s) * 0.8)(D, 3 * D)), 'wo': _w((lambda *s: _rng.normal(s) * 0.05)(D, D))}
    _A_in = _A_setup()

    def _B_setup():
        B, S, Dm = (1, 2048, 512)
        H, Dh = (32, 128)
        M, seg = (8, 32)
        seg = min(seg, S)
        S = S // seg * seg
        return {'x': _w((lambda *s: _rng.normal(s) * 0.05)(B, S, Dm)), 'mem0': _w((lambda *s: _rng.normal(s) * 0.8)(B, M, Dm)), 'Wq': _w((lambda *s: _rng.normal(s) * 1.6)(Dm, H, Dh) * Dm ** (-0.5)), 'Wk': _w((lambda *s: _rng.normal(s) * 1.6)(Dm, H, Dh) * Dm ** (-0.5)), 'Wv': _w((lambda *s: _rng.normal(s) * 0.8)(Dm, H, Dh) * Dm ** (-0.5)), 'Wo': _w((lambda *s: _rng.normal(s) * 0.8)(H, Dh, Dm) * (H * Dh) ** (-0.5)), 'seg_len': seg}
    _B_in = _B_setup()
    return {'A_x': _A_in['x'], 'A_wqkv': _A_in['wqkv'], 'A_wo': _A_in['wo'], 'B_x': _B_in['x'], 'B_mem0': _B_in['mem0'], 'B_Wq': _B_in['Wq'], 'B_Wk': _B_in['Wk'], 'B_Wv': _B_in['Wv'], 'B_Wo': _B_in['Wo'], 'B_seg_len': _B_in['seg_len'], 'gate_w': _w((lambda *s: _rng.normal(s) * 0.05)(512) * 16.0)}

def reference(A_x, A_wqkv, A_wo, B_x, B_mem0, B_Wq, B_Wk, B_Wv, B_Wo, B_seg_len, gate_w):

    def _A_ref(x, wqkv, wo):
        B, S, D = x.shape
        H = 32
        Dh = D // H
        qkv = (lambda x, *d: x.transpose(*d))((x @ wqkv).reshape(B, S, 3, H, Dh), 2, 0, 3, 1, 4)
        q, k, v = (qkv[0], qkv[1], qkv[2])
        scores = jnp.einsum('bhqd,bhkd->bhqk', q, k) * Dh ** (-0.5)
        p = _softmax(scores, axis=-1)
        o = jnp.einsum('bhqk,bhkd->bhqd', p, v)
        return (lambda x, *d: x.transpose(*d))(o, 0, 2, 1, 3).reshape(B, S, D) @ wo

    def _B_ref(x, mem0, Wq, Wk, Wv, Wo, seg_len):
        B, S, Dm = x.shape
        H, Dh = (Wq.shape[1], Wq.shape[2])
        M = mem0.shape[1]
        scale = Dh ** (-0.5)
        n_seg = S // seg_len
        L = M + seg_len
        idx = jnp.arange(L)
        mask = (idx[:, None] < M) | (idx[:, None] >= idx[None, :])
        mem = mem0
        outs = []
        for s in range(n_seg):
            xs = x[:, s * seg_len:(s + 1) * seg_len, :].copy()
            h = jnp.concatenate([mem, xs], axis=1)
            q = jnp.einsum('btd,dhe->bhte', h, Wq)
            k = jnp.einsum('btd,dhe->bhte', h, Wk)
            v = jnp.einsum('btd,dhe->bhte', h, Wv)
            scores = jnp.einsum('bhqe,bhke->bhqk', q, k) * scale
            scores = jnp.where(mask[None, None], scores, -1000000000.0)
            p = _softmax(scores, axis=-1)
            o = jnp.einsum('bhqk,bhke->bhqe', p, v)
            o = jnp.einsum('bhte,hed->btd', o, Wo)
            mem = o[:, :M, :].copy()
            outs.append(o[:, M:, :])
        return jnp.concatenate(outs, axis=1)
    x = A_x
    g = _sigmoid((x * gate_w).sum(-1, keepdims=True))
    a = _A_ref(x, A_wqkv, A_wo)
    b = _B_ref(x, B_mem0, B_Wq, B_Wk, B_Wv, B_Wo, B_seg_len)
    return g * a + (1 - g) * b
```

```python
import functools

import jax
import jax.numpy as jnp
import numpy as np
from jax import lax
from jax.experimental import pallas as pl
from jax.experimental.pallas import tpu as pltpu

F32 = jnp.float32
BF16 = jnp.bfloat16
U32 = jnp.uint32
LOG2E = float(np.log2(np.e))

HA = 32
QB = 128
KG = 256
KC = 64
LAG = 2
NSB = 4
UNR = 32
HG = 2
PB = 2
NB = 4
FILL = 1
BL1 = 1; BL2 = 4; BL3 = 4


def _nt(a, b):
    return lax.dot_general(a, b, (((1,), (1,)), ((), ())), preferred_element_type=F32)


def _nn(a, b):
    return lax.dot_general(a, b, (((1,), (0,)), ((), ())), preferred_element_type=F32)


def _u32(v):
    return pltpu.bitcast(v, U32)


def _bf(v):
    return pltpu.bitcast(v, BF16)


def _kernel(z_ref, mem0_ref, gw_ref,
            x_hbm, wqkv_hbm, wo_hbm, bq_hbm, bk_hbm, bv_hbm, bo_hbm,
            out_hbm,
            x_ref, wqkv_ref, wo_ref, stage_ref, stage_o,
            wq_u, wk_u, wv_u, wo_u, wqvT_u, awo_u,
            qt_u, kh_u, vt_u, ot_u, g_ref, ob_ref, sems, xsems, osems, *s_refs,
            S, D, SEG, M, HB, EB):
    z0 = z_ref[0]
    z1 = z_ref[1]
    DH = D // HA
    NQB = S // QB
    L = M + SEG
    NI = HA * NQB
    NIT = NI // UNR

    DC = D // NIT
    XR = PB * QB

    def wcp(i):
        return pltpu.make_async_copy(wqkv_hbm.at[:, pl.ds(i * D, D)], wqkv_ref.at[:, pl.ds(i * D, D)], sems.at[i])

    def xcp(t):
        rows = pl.ds(pl.multiple_of(t * XR, XR), XR)
        return pltpu.make_async_copy(x_hbm.at[rows], x_ref.at[rows], xsems.at[t])

    cp_wo = pltpu.make_async_copy(wo_hbm, wo_ref, sems.at[3])
    cp_b0 = [pltpu.make_async_copy(src.at[pl.ds(0, DC)], stage_ref.at[i, pl.ds(0, DC)], sems.at[4 + i])
             for i, src in enumerate((bq_hbm, bk_hbm, bv_hbm))]
    cp_b0.append(pltpu.make_async_copy(bo_hbm.at[pl.ds(0, HB // NIT)], stage_o.at[pl.ds(0, HB // NIT)], sems.at[7]))
    cp_b1 = [pltpu.make_async_copy(src.at[pl.ds(DC, D - DC)], stage_ref.at[i, pl.ds(DC, D - DC)], sems.at[8 + i])
             for i, src in enumerate((bq_hbm, bk_hbm, bv_hbm))]
    cp_b1.append(pltpu.make_async_copy(bo_hbm.at[pl.ds(HB // NIT, HB - HB // NIT)],
                                       stage_o.at[pl.ds(HB // NIT, HB - HB // NIT)], sems.at[11]))
    for i in (0, 2, 1):
        wcp(i).start()

    wcp(0).wait()
    for t in range(S // XR):
        xcp(t).start()
    wqvT_u[0] = _u32(wqkv_ref[:, 0:D].T)
    wcp(2).wait()
    for c in cp_b0 + cp_b1:
        c.start()
    cp_wo.start()
    wqvT_u[1] = _u32(wqkv_ref[:, 2 * D:3 * D].T)
    wcp(1).wait()
    qscale = (DH ** -0.5) * LOG2E
    gw = gw_ref[...].astype(F32).reshape(1, D)

    def proj_block(j):
        r0 = pl.multiple_of(j * QB, QB)
        xc = x_ref[pl.ds(r0, QB), :]
        kc = _u32(_nn(xc, wqkv_ref[:, D:2 * D]).astype(BF16))
        for gcol in range(D // 128):
            tile = kc[:, gcol * 128:(gcol + 1) * 128]
            for jj in range(128 // DH):
                h = gcol * (128 // DH) + jj
                kh_u[h, pl.ds(pl.multiple_of(j * (QB // 2), QB // 2), QB // 2), :] = (
                    tile if jj == 0 else pltpu.roll(tile, 128 - jj * DH, 1))
        gl = jnp.sum(xc.astype(F32) * gw, axis=-1, keepdims=True)
        g_ref[pl.ds(r0, QB), :] = jnp.broadcast_to(1.0 / (1.0 + jnp.exp(-gl)), (QB, 128))
        qt_u[j] = _u32((_nt(_bf(wqvT_u[0]), xc) * qscale).astype(BF16))
        vt_u[j] = _u32(_nt(_bf(wqvT_u[1]), xc).astype(BF16))

    def proj_body(t, c):
        xcp(t).wait()
        for p in range(PB):
            proj_block(t * PB + p)
        return c

    lax.fori_loop(0, NQB // PB, proj_body, 0)

    WP = D // 2 + 1

    def relayout(t):
        for wi, dst in enumerate((wq_u, wk_u, wv_u)):
            wu = _u32(stage_ref[wi, pl.ds(pl.multiple_of(t * DC, DC), DC)].reshape(DC * HB, EB))
            for i in range(DC // 2):
                ev = wu[(2 * i) * (HB // 2):(2 * i + 1) * (HB // 2), :]
                od = wu[(2 * i + 1) * (HB // 2):(2 * i + 2) * (HB // 2), :]
                lo = (ev & jnp.uint32(0xffff)) | (od << 16)
                hi = (ev >> 16) | (od & jnp.uint32(0xffff0000))
                r = t * (DC // 2) + i
                dst[pl.ds(r, HB // 2, stride=2 * WP), :] = lo
                dst[pl.ds(r + WP, HB // 2, stride=2 * WP), :] = hi
        for hh in range(HB // NIT):
            h = t * (HB // NIT) + hh
            wo_u[pl.ds(pl.multiple_of(h * (EB // 2), EB // 2), EB // 2), :] = _u32(stage_o[h])

    def qk_group(h, qt, g, sref, m):
        for c in range(KG // KC):
            r0 = g * KG + c * KC
            st = _nn(_bf(kh_u[h, r0 // 2:(r0 + KC) // 2, :])[:, 0:DH], qt)
            sref[z0, r0:r0 + KC, :] = st
            for t in range(KC // 8):
                v = st[t * 8:(t + 1) * 8, :]
                m = v if m is None else jnp.maximum(m, v)
        return m

    def pv_group(h, m, g, sref, acc):
        e = jnp.exp2(sref[z1, g * KG:(g + 1) * KG, :] - m)
        nb = KG // QB
        hr = pl.ds(pl.multiple_of(h * (DH // 2), DH // 2), DH // 2)
        vt = jnp.concatenate([_bf(vt_u[g * nb + b, hr, :]) for b in range(nb)], axis=1)
        parts = [e[t * 8:(t + 1) * 8, :] for t in range(KG // 8)]
        while len(parts) > 1:
            parts = [parts[a] + parts[a + 1] for a in range(0, len(parts), 2)]
        o = _nn(vt, e.astype(BF16))
        return (o, parts[0]) if acc is None else (acc[0] + o, acc[1] + parts[0])

    def load_qt(i):
        h = i % HA
        return _bf(qt_u[i // HA, pl.ds(pl.multiple_of(h * (DH // 2), DH // 2), DH // 2), :])

    def fin(m):
        return jnp.max(m, axis=0, keepdims=True)

    def a_step(i, u, ms):
        sw = s_refs[(u + LAG) % NSB]
        sr = s_refs[u % NSB]
        inext = jnp.minimum(i + LAG, NI - 1)
        hq = inext % HA
        qt = load_qt(inext)
        h = i % HA
        mn = None
        acc = None
        for g in range(S // KG):
            mn = qk_group(hq, qt, g, sw, mn)
            acc = pv_group(h, ms[0], g, sr, acc)
        o = acc[0] * (1.0 / jnp.sum(acc[1], axis=0, keepdims=True))
        ot_u[i // HA, pl.ds(pl.multiple_of(h * (DH // 2), DH // 2), DH // 2), :] = _u32(o.astype(BF16))
        return ms[1:] + (fin(mn),)

    ms = ()
    for j in range(LAG):
        qt = load_qt(j)
        mn = None
        for g in range(S // KG):
            mn = qk_group(j, qt, g, s_refs[j], mn)
        ms = ms + (fin(mn),)

    for c in cp_b0:
        c.wait()
    if not FILL:
        for c in cp_b1:
            c.wait()

    def a_body(t, ms):
        if FILL:
            @pl.when(t == 1)
            def _():
                for c in cp_b1:
                    c.wait()
        for u in range(UNR):
            ms = a_step(t * UNR + u, u, ms)
        if FILL:
            relayout(t)
        return ms

    lax.fori_loop(0, NIT, a_body, ms)
    if not FILL:
        def rl(t, c):
            relayout(t)
            return c
        lax.fori_loop(0, NIT, rl, 0)

    cp_wo.wait()
    awo_u[...] = _u32(wo_ref[...])

    row = lax.broadcasted_iota(jnp.int32, (L, L), 0)
    col = lax.broadcasted_iota(jnp.int32, (L, L), 1)
    mask = (row < M) | (row >= col)
    sscale = (EB ** -0.5) * LOG2E
    NG = HB // HG

    def b_proj(h40, g):
        out = []
        for j in range(HG):
            r0 = (g * HG + j) * WP
            q = _nn(h40, _bf(wq_u[r0:r0 + D // 2, :]))
            k = _nn(h40, _bf(wk_u[r0:r0 + D // 2, :])).astype(BF16)
            v = _nn(h40, _bf(wv_u[r0:r0 + D // 2, :])).astype(BF16)
            out.append((q, k, v))
        return out

    def b_scores(qkv):
        out = []
        for q, k, v in qkv:
            s = jnp.where(mask, _nt(q, k) * sscale, -1e9 * LOG2E)
            p = jnp.exp2(s - jnp.max(s, axis=-1, keepdims=True))
            out.append((p, 1.0 / jnp.sum(p, axis=-1, keepdims=True), v))
        return out

    def b_pv(prv):
        return [_nn(p, v) * r for p, r, v in prv]

    def b_out(os_, g, acc):
        r0 = g * HG * EB // 2
        y = _nn(jnp.concatenate(os_, axis=1), _bf(wo_u[r0:r0 + HG * EB // 2, :]))
        return y if acc is None else acc + y

    def b_step(s, mem, a_rows):
        r0 = pl.multiple_of(s * SEG, SEG)
        h40 = jnp.concatenate([mem, x_ref[pl.ds(r0, SEG), :].astype(F32)], axis=0)
        qkv, sc, ov = {}, {}, {}
        acc = None
        for t in range(NG + BL1 + BL2 + BL3):
            if t < NG:
                qkv[t] = b_proj(h40, t)
            g = t - BL1
            if 0 <= g < NG:
                sc[g] = b_scores(qkv.pop(g))
            g = t - BL1 - BL2
            if 0 <= g < NG:
                ov[g] = b_pv(sc.pop(g))
            g = t - BL1 - BL2 - BL3
            if 0 <= g < NG:
                acc = b_out(ov.pop(g), g, acc)
        a = _nn(a_rows, _bf(awo_u[...]))
        g = g_ref[pl.ds(r0, SEG), :]
        parts = []
        for c in range(D // 128):
            sl = slice(c * 128, (c + 1) * 128)
            b = acc[M:, sl]
            parts.append(b + g * (a[:, sl] - b))
        ob_ref[pl.ds(r0, SEG), :] = jnp.concatenate(parts, axis=1).astype(BF16)
        return acc[:M, :].astype(BF16).astype(F32)

    def b_body(t, mem):
        on = _bf(ot_u[t]).T
        for u in range(NB):
            mem = b_step(t * NB + u, mem, on[u * SEG:(u + 1) * SEG, :])
        r0 = pl.multiple_of(t * QB, QB)
        pltpu.make_async_copy(ob_ref.at[pl.ds(r0, QB)], out_hbm.at[pl.ds(r0, QB)], osems.at[t]).start()
        return mem

    lax.fori_loop(0, NQB, b_body, mem0_ref[...].astype(F32))
    for t in range(NQB):
        pltpu.make_async_copy(ob_ref.at[pl.ds(t * QB, QB)], out_hbm.at[pl.ds(t * QB, QB)], osems.at[t]).wait()


@functools.partial(jax.jit, static_argnames=("B_seg_len",))
def pallas_gated_mix__mha_block__memory_aug_recurrent_mem_tr__prompt_kernel(
    A_x, A_wqkv, A_wo, B_x, B_mem0, B_Wq, B_Wk, B_Wv, B_Wo, B_seg_len, gate_w):
    del B_x
    _, S, D = A_x.shape
    M = B_mem0.shape[1]
    _, HB, EB = B_Wq.shape
    SEG = int(B_seg_len)
    assert SEG * NB == QB
    NIT = HA * (S // QB) // UNR
    DC = D // NIT
    kern = functools.partial(_kernel, S=S, D=D, SEG=SEG, M=M, HB=HB, EB=EB)
    any_spec = pl.BlockSpec(memory_space=pl.ANY)
    out = pl.pallas_call(
        kern,
        out_shape=jax.ShapeDtypeStruct((S, D), A_x.dtype),
        in_specs=[pl.BlockSpec(memory_space=pltpu.SMEM),
                  pl.BlockSpec(memory_space=pltpu.VMEM),
                  pl.BlockSpec(memory_space=pltpu.VMEM)] + [any_spec] * 7,
        out_specs=any_spec,
        scratch_shapes=[
            pltpu.VMEM((S, D), BF16),
            pltpu.VMEM((D, 3 * D), BF16),
            pltpu.VMEM((D, D), BF16),
            pltpu.VMEM((3, D, HB, EB), BF16),
            pltpu.VMEM((HB, EB, D), BF16),
            pltpu.VMEM((HB * (D // 2 + 1), EB), U32),
            pltpu.VMEM((HB * (D // 2 + 1), EB), U32),
            pltpu.VMEM((HB * (D // 2 + 1), EB), U32),
            pltpu.VMEM((HB * EB // 2, D), U32),
            pltpu.VMEM((2, D // 2, D), U32),
            pltpu.VMEM((D // 2, D), U32),
            pltpu.VMEM((S // QB, D // 2, QB), U32),
            pltpu.VMEM((HA, S // 2, 128), U32),
            pltpu.VMEM((S // QB, D // 2, QB), U32),
            pltpu.VMEM((S // QB, D // 2, QB), U32),
            pltpu.VMEM((S, 128), F32),
            pltpu.VMEM((S, D), BF16),
            pltpu.SemaphoreType.DMA((12,)),
            pltpu.SemaphoreType.DMA((S // (PB * QB),)),
            pltpu.SemaphoreType.DMA((S // QB,)),
        ] + [pltpu.VMEM((1, S, QB), F32)] * NSB,
        compiler_params=pltpu.CompilerParams(vmem_limit_bytes=110 * 1024 * 1024),
    )(jnp.zeros((2,), jnp.int32), B_mem0.reshape(M, D), gate_w,
      A_x.reshape(S, D), A_wqkv, A_wo, B_Wq, B_Wk, B_Wv, B_Wo)
    return out.reshape(1, S, D)
```

```python
import functools

import jax
import jax.numpy as jnp
import numpy as np
from jax import lax
from jax.experimental import pallas as pl
from jax.experimental.pallas import tpu as pltpu

F32 = jnp.float32
BF16 = jnp.bfloat16
U32 = jnp.uint32
LOG2E = float(np.log2(np.e))

HA = 32
QB = 128
KG = 512
KC = 128
LAG = 2
NSB = 4
UNR = 32
PB = 2
HG = 2
BL1, BL2, BL3 = 1, 4, 2


def _nt(a, b):
    return lax.dot_general(a, b, (((1,), (1,)), ((), ())), preferred_element_type=F32)


def _nn(a, b):
    return lax.dot_general(a, b, (((1,), (0,)), ((), ())), preferred_element_type=F32)


def _u32(v):
    return pltpu.bitcast(v, U32)


def _bf(v):
    return pltpu.bitcast(v, BF16)


def _kernel(z_ref, mem0_hbm, gw_hbm,
            x_hbm, wqkv_hbm, wo_hbm, bq_hbm, bk_hbm, bv_hbm, bo_hbm,
            out_hbm,
            x_ref, wqkv_ref, wo_ref, stage_ref, bo_ref,
            wq_u, wk_u, wv_u, wqvT_u,
            qt_u, kh_u, vt_u, ot_u, g_ref, ob_ref, sems, xsems, osems, *rest,
            S, D, SEG, M, HB, EB):
    s_refs, (mem0_ref, gw_ref) = rest[:NSB], rest[NSB:]
    DH = D // HA
    NQB = S // QB
    NI = HA * NQB
    NIT = NI // UNR
    DC = D // NIT
    XR = PB * QB
    WP = D // 2 + 1
    NB = QB // SEG
    L = M + SEG
    z0 = z_ref[0]
    z1 = z_ref[1]

    def wcp(i):
        cols = pl.ds(i * D, D)
        return pltpu.make_async_copy(wqkv_hbm.at[:, cols], wqkv_ref.at[:, cols], sems.at[i])

    def xcp(t):
        rows = pl.ds(pl.multiple_of(t * XR, XR), XR)
        return pltpu.make_async_copy(x_hbm.at[rows], x_ref.at[rows], xsems.at[t])

    def ocp(t):
        rows = pl.ds(pl.multiple_of(t * QB, QB), QB)
        return pltpu.make_async_copy(ob_ref.at[rows], out_hbm.at[rows], osems.at[t])

    b_src = (bq_hbm, bk_hbm, bv_hbm)
    cp_head = [pltpu.make_async_copy(src.at[pl.ds(0, DC)], stage_ref.at[i, pl.ds(0, DC)], sems.at[3 + i])
               for i, src in enumerate(b_src)]
    cp_rest = [pltpu.make_async_copy(src.at[pl.ds(DC, D - DC)], stage_ref.at[i, pl.ds(DC, D - DC)],
                                     sems.at[6 + i])
               for i, src in enumerate(b_src)]
    cp_bo = pltpu.make_async_copy(bo_hbm, bo_ref, sems.at[9])
    cp_wo = pltpu.make_async_copy(wo_hbm, wo_ref, sems.at[10])
    cp_gw = pltpu.make_async_copy(gw_hbm, gw_ref, sems.at[11])
    cp_mem = pltpu.make_async_copy(mem0_hbm, mem0_ref, sems.at[12])

    for i in (0, 2, 1):
        wcp(i).start()
    cp_gw.start()
    wcp(0).wait()
    for t in range(S // XR):
        xcp(t).start()
    wqvT_u[0] = _u32(wqkv_ref[:, 0:D].T)
    wcp(2).wait()
    for c in cp_head + cp_rest:
        c.start()
    cp_bo.start()
    cp_wo.start()
    cp_mem.start()
    wqvT_u[1] = _u32(wqkv_ref[:, 2 * D:3 * D].T)
    wcp(1).wait()

    qscale = (DH ** -0.5) * LOG2E
    cp_gw.wait()
    gw = gw_ref[...].astype(F32).reshape(1, D)

    def proj_block(j):
        r0 = pl.multiple_of(j * QB, QB)
        xc = x_ref[pl.ds(r0, QB), :]
        kc = _u32(_nn(xc, wqkv_ref[:, D:2 * D]).astype(BF16))
        for gcol in range(D // 128):
            tile = kc[:, gcol * 128:(gcol + 1) * 128]
            for jj in range(128 // DH):
                h = gcol * (128 // DH) + jj
                kh_u[h, pl.ds(pl.multiple_of(j * (QB // 2), QB // 2), QB // 2), :] = (
                    tile if jj == 0 else pltpu.roll(tile, 128 - jj * DH, 1))
        gl = jnp.sum(xc.astype(F32) * gw, axis=-1, keepdims=True)
        g_ref[pl.ds(r0, QB), :] = jnp.broadcast_to(1.0 / (1.0 + jnp.exp(-gl)), (QB, 128))
        qt_u[j] = _u32((_nt(_bf(wqvT_u[0]), xc) * qscale).astype(BF16))
        vt_u[j] = _u32(_nt(_bf(wqvT_u[1]), xc).astype(BF16))

    def proj_body(t, carry):
        xcp(t).wait()
        for p in range(PB):
            proj_block(t * PB + p)
        return carry

    lax.fori_loop(0, S // XR, proj_body, 0)

    def relayout(t):
        for wi, dst in enumerate((wq_u, wk_u, wv_u)):
            wu = _u32(stage_ref[wi, pl.ds(pl.multiple_of(t * DC, DC), DC)].reshape(DC * HB, EB))
            for i in range(DC // 2):
                ev = wu[(2 * i) * (HB // 2):(2 * i + 1) * (HB // 2), :]
                od = wu[(2 * i + 1) * (HB // 2):(2 * i + 2) * (HB // 2), :]
                r = t * (DC // 2) + i
                dst[pl.ds(r, HB // 2, stride=2 * WP), :] = (ev & jnp.uint32(0xffff)) | (od << 16)
                dst[pl.ds(r + WP, HB // 2, stride=2 * WP), :] = (ev >> 16) | (od & jnp.uint32(0xffff0000))

    def head_rows(h):
        return pl.ds(pl.multiple_of(h * (DH // 2), DH // 2), DH // 2)

    def qk_group(h, qt, g, sref, m):
        for c in range(KG // KC):
            r0 = g * KG + c * KC
            st = _nn(_bf(kh_u[h, r0 // 2:(r0 + KC) // 2, :])[:, 0:DH], qt)
            sref[z0, r0:r0 + KC, :] = st
            v = jnp.max(st.reshape(KC // 8, 8, QB), axis=0)
            m = v if m is None else jnp.maximum(m, v)
        return m

    def pv_group(h, m, g, sref, acc):
        e = jnp.exp2(sref[z1, g * KG:(g + 1) * KG, :] - m)
        nb = KG // QB
        vt = jnp.concatenate([_bf(vt_u[g * nb + b, head_rows(h), :]) for b in range(nb)], axis=1)
        ls = e
        while ls.shape[0] > 8:
            ls = ls.reshape(ls.shape[0] // 16, 2, 8, QB)
            ls = (ls[:, 0] + ls[:, 1]).reshape(-1, QB)
        o = _nn(vt, e.astype(BF16))
        return (o, ls) if acc is None else (acc[0] + o, acc[1] + ls)

    def qk_item(i, sref):
        h = i % HA
        qt = _bf(qt_u[i // HA, head_rows(h), :])
        return lambda g, m: qk_group(h, qt, g, sref, m)

    def row_max(m):
        return jnp.max(m, axis=0, keepdims=True)

    def a_step(i, u, ms):
        qk = qk_item(jnp.minimum(i + LAG, NI - 1), s_refs[(u + LAG) % NSB])
        h = i % HA
        mn = None
        acc = None
        for g in range(S // KG):
            mn = qk(g, mn)
            acc = pv_group(h, ms[0], g, s_refs[u % NSB], acc)
        o = acc[0] * (1.0 / jnp.sum(acc[1], axis=0, keepdims=True))
        ot_u[i // HA, head_rows(h), :] = _u32(o.astype(BF16))
        return ms[1:] + (row_max(mn),)

    ms = ()
    for j in range(LAG):
        qk = qk_item(j, s_refs[j])
        mn = None
        for g in range(S // KG):
            mn = qk(g, mn)
        ms = ms + (row_max(mn),)

    for c in cp_head:
        c.wait()

    def a_body(t, ms):
        @pl.when(t == 1)
        def _():
            for c in cp_rest:
                c.wait()

        for u in range(UNR):
            ms = a_step(t * UNR + u, u, ms)
        relayout(t)
        return ms

    lax.fori_loop(0, NIT, a_body, ms)
    cp_bo.wait()
    cp_wo.wait()
    cp_mem.wait()

    row = lax.broadcasted_iota(jnp.int32, (L, L), 0)
    col = lax.broadcasted_iota(jnp.int32, (L, L), 1)
    mask = (row < M) | (row >= col)
    sscale = (EB ** -0.5) * LOG2E
    NG = HB // HG

    def b_proj(h40, g):
        out = []
        for j in range(HG):
            r0 = (g * HG + j) * WP
            q = _nn(h40, _bf(wq_u[r0:r0 + D // 2, :]))
            k = _nn(h40, _bf(wk_u[r0:r0 + D // 2, :])).astype(BF16)
            v = _nn(h40, _bf(wv_u[r0:r0 + D // 2, :])).astype(BF16)
            out.append((q, k, v))
        return out

    def b_scores(qkv):
        out = []
        for q, k, v in qkv:
            s = jnp.where(mask, _nt(q, k) * sscale, -1e9 * LOG2E)
            p = jnp.exp2(s - jnp.max(s, axis=-1, keepdims=True))
            out.append((p, 1.0 / jnp.sum(p, axis=-1, keepdims=True), v))
        return out

    def b_pv(prv):
        return [_nn(p, v) * r for p, r, v in prv]

    def b_out(os_, g, acc):
        y = _nn(jnp.concatenate(os_, axis=1), bo_ref[g * HG:(g + 1) * HG].reshape(HG * EB, D))
        return y if acc is None else acc + y

    def b_step(s, mem, o_rows):
        r0 = pl.multiple_of(s * SEG, SEG)
        h40 = jnp.concatenate([mem, x_ref[pl.ds(r0, SEG), :].astype(F32)], axis=0)
        qkv, sc, ov = {}, {}, {}
        acc = None
        for t in range(NG + BL1 + BL2 + BL3):
            if t < NG:
                qkv[t] = b_proj(h40, t)
            g = t - BL1
            if 0 <= g < NG:
                sc[g] = b_scores(qkv.pop(g))
            g = t - BL1 - BL2
            if 0 <= g < NG:
                ov[g] = b_pv(sc.pop(g))
            g = t - BL1 - BL2 - BL3
            if 0 <= g < NG:
                acc = b_out(ov.pop(g), g, acc)
        a = _nn(o_rows, wo_ref[...])
        gate = g_ref[pl.ds(r0, SEG), :]
        parts = []
        for c in range(D // 128):
            sl = slice(c * 128, (c + 1) * 128)
            b = acc[M:, sl]
            parts.append(b + gate * (a[:, sl] - b))
        ob_ref[pl.ds(r0, SEG), :] = jnp.concatenate(parts, axis=1).astype(BF16)
        return acc[:M, :].astype(BF16).astype(F32)

    def b_body(t, mem):
        o_nat = _bf(ot_u[t]).T
        for u in range(NB):
            mem = b_step(t * NB + u, mem, o_nat[u * SEG:(u + 1) * SEG, :])
        ocp(t).start()
        return mem

    lax.fori_loop(0, NQB, b_body, mem0_ref[...].astype(F32))
    for t in range(NQB):
        ocp(t).wait()


@functools.partial(jax.jit, static_argnames=("B_seg_len",))
def pallas_gated_mix__mha_block__memory_aug_recurrent_mem_tr__prompt_kernel(
    A_x: jax.Array,
    A_wqkv: jax.Array,
    A_wo: jax.Array,
    B_x: jax.Array,
    B_mem0: jax.Array,
    B_Wq: jax.Array,
    B_Wk: jax.Array,
    B_Wv: jax.Array,
    B_Wo: jax.Array,
    B_seg_len: int,
    gate_w: jax.Array,
):
    del B_x
    _, S, D = A_x.shape
    M = B_mem0.shape[1]
    _, HB, EB = B_Wq.shape
    SEG = int(B_seg_len)
    assert QB % SEG == 0 and S % (PB * QB) == 0 and S % KG == 0
    assert (HA * S // QB) % UNR == 0 and HA * S // QB >= 2 * UNR
    wrows = ((HB + 2) * (D // 2 + 1) + 31) // 32 * 32
    any_spec = pl.BlockSpec(memory_space=pl.ANY)
    out = pl.pallas_call(
        functools.partial(_kernel, S=S, D=D, SEG=SEG, M=M, HB=HB, EB=EB),
        out_shape=jax.ShapeDtypeStruct((S, D), A_x.dtype),
        in_specs=[pl.BlockSpec(memory_space=pltpu.SMEM),
                  ] + [any_spec] * 9,
        out_specs=any_spec,
        scratch_shapes=[
            pltpu.VMEM((S, D), BF16),
            pltpu.VMEM((D, 3 * D), BF16),
            pltpu.VMEM((D, D), BF16),
            pltpu.VMEM((3, D, HB, EB), BF16),
            pltpu.VMEM((HB, EB, D), BF16),
            pltpu.VMEM((wrows, EB), U32),
            pltpu.VMEM((wrows, EB), U32),
            pltpu.VMEM((wrows, EB), U32),
            pltpu.VMEM((2, D // 2, D), U32),
            pltpu.VMEM((S // QB, D // 2, QB), U32),
            pltpu.VMEM((HA, S // 2, 128), U32),
            pltpu.VMEM((S // QB, D // 2, QB), U32),
            pltpu.VMEM((S // QB, D // 2, QB), U32),
            pltpu.VMEM((S, 128), F32),
            pltpu.VMEM((S, D), BF16),
            pltpu.SemaphoreType.DMA((13,)),
            pltpu.SemaphoreType.DMA((S // (PB * QB),)),
            pltpu.SemaphoreType.DMA((S // QB,)),
        ] + [pltpu.VMEM((1, S, QB), F32)] * NSB + [
            pltpu.VMEM((M, D), BF16),
            pltpu.VMEM((D,), BF16),
        ],
        compiler_params=pltpu.CompilerParams(vmem_limit_bytes=110 * 1024 * 1024),
    )(jnp.zeros((2,), jnp.int32), B_mem0.reshape(M, D), gate_w,
      A_x.reshape(S, D), A_wqkv, A_wo, B_Wq, B_Wk, B_Wv, B_Wo)
    return out.reshape(1, S, D)
```
